```python
import os as _os
_os.environ.setdefault("JAX_PLATFORMS", "cpu")
import jax
import jax.numpy as jnp

def _softmax(x, axis=-1):
    return jax.nn.softmax(x, axis=axis)
def _gelu(x):
    return jax.nn.gelu(x, approximate=True)
def _silu(x):
    return jax.nn.silu(x)
def _sigmoid(x):
    return jax.nn.sigmoid(x)
def _layernorm(x, axis=-1, eps=1e-5):
    m = jnp.mean(x, axis=axis, keepdims=True)
    v = jnp.var(x, axis=axis, keepdims=True)
    return (x - m) / jnp.sqrt(v + eps)
def _scatter_add(tgt, idx, src, axis=0):
    return tgt.at[idx].add(src)
def _segment_sum(src, seg, n):
    return jax.ops.segment_sum(src, seg, n)
class _Rng:
    def __init__(self, key):
        self._k = key
    def _next(self):
        self._k, sub = jax.random.split(self._k)
        return sub
    def normal(self, shape):
        return jax.random.normal(self._next(), shape, dtype=jnp.bfloat16)
    def randint(self, lo, hi, shape):
        return jax.random.randint(self._next(), shape, lo, hi, dtype=jnp.int32)
    def uniform(self, shape, lo=0.0, hi=1.0):
        return jax.random.uniform(self._next(), shape, jnp.bfloat16, lo, hi)
    def permutation(self, n):
        return jax.random.permutation(self._next(), n)


kernel_name = 'concat_heads__spectral_gfnet__mha_block__prompt'

def setup_inputs():
    _rng = _Rng(jax.random.key(int.from_bytes(__import__("os").urandom(4), "little")))
    _w = (lambda a: (lambda t: t.astype(jnp.bfloat16) if jnp.issubdtype(t.dtype, jnp.floating) else t)(jnp.asarray(a)))
    def _A_setup():
        B, S, D = 1, 2048, 576
        Df = D // 2 + 1
        return {
            "x": _w((lambda *s: _rng.normal(s) * 0.05)(B, S, D)),
            "w_r": _w((lambda *s: _rng.normal(s) * 0.05)(S, Df) * 0.02),
            "w_i": _w((lambda *s: _rng.normal(s) * 0.05)(S, Df) * 0.02),
        }
    _A_in = _A_setup()

    def _B_setup():
        B, S, D, H = 1, 2048, 576, 32
        return {
            "x": _w((lambda *s: _rng.normal(s) * 0.1)(B, S, D)),
            "wqkv": _w((lambda *s: _rng.normal(s) * 0.1)(D, 3 * D)),
            "wo": _w((lambda *s: _rng.normal(s) * 0.05)(D, D)),
        }
    _B_in = _B_setup()

    return {
        "A_x": _A_in["x"],
        "A_w_r": _A_in["w_r"],
        "A_w_i": _A_in["w_i"],
        "B_x": _B_in["x"],
        "B_wqkv": _B_in["wqkv"],
        "B_wo": _B_in["wo"],
    }

def reference(A_x, A_w_r, A_w_i, B_x, B_wqkv, B_wo):
    def _A_ref(x, w_r, w_i):
        B, S, D = x.shape
        X = (lambda x, axes=(-2,-1): jnp.fft.rfft2(x.astype(jnp.float32), axes=axes))(x, axes=(-2, -1))
        W = w_r + 1j * w_i
        X = X * W
        y = (lambda x, s, axes=(-2,-1): jnp.fft.irfft2(x, s=s, axes=axes).astype(jnp.bfloat16))(X, (S, D), axes=(-2, -1))
        return y

    def _B_ref(x, wqkv, wo):
        B, S, D = x.shape
        H = 32
        Dh = D // H
        qkv = (lambda x, *d: x.transpose(*d))((x @ wqkv).reshape(B, S, 3, H, Dh), 2, 0, 3, 1, 4)
        q, k, v = qkv[0], qkv[1], qkv[2]
        scores = jnp.einsum("bhqd,bhkd->bhqk", q, k) * (Dh ** -0.5)
        p = _softmax(scores, axis=-1)
        o = jnp.einsum("bhqk,bhkd->bhqd", p, v)
        return (lambda x, *d: x.transpose(*d))(o, 0, 2, 1, 3).reshape(B, S, D) @ wo

    a = _A_ref(A_x, A_w_r, A_w_i)
    b = _B_ref(B_x, B_wqkv, B_wo)
    return jnp.concatenate([a, b], axis=-1)
```

```python
import functools
import numpy as np, jax, jax.numpy as jnp, ml_dtypes
from jax import lax
from jax.experimental import pallas as pl
from jax.experimental.pallas import tpu as pltpu

f32 = jnp.float32; bf = jnp.bfloat16; u32 = jnp.uint32
S, D, H, DH = 2048, 576, 32, 18
DF = D // 2 + 1
FP = 296
NN = (((1,), (0,)), ((), ()))
CQ = float(DH ** -0.5 * np.log2(np.e))
T_SAFE = 40.0

def _consts():
    nb = ml_dtypes.bfloat16
    f = np.arange(DF)[:, None].astype(np.float64); d = np.arange(D)[None, :].astype(np.float64)
    ang = 2 * np.pi * ((f * d) % D) / D
    ft = np.zeros((2 * FP, D)); ft[:DF] = np.cos(ang); ft[FP:FP + DF] = -np.sin(ang)
    cf = np.full((DF, 1), 2.0); cf[0] = 1.0; cf[-1] = 1.0
    gt = np.zeros((2 * FP, D)); gt[:DF] = cf * np.cos(ang); gt[FP:FP + DF] = -cf * np.sin(ang)
    gt = gt.T / (D * S)
    n = np.arange(128)[:, None].astype(np.float64); k = np.arange(128)[None, :].astype(np.float64)
    a2 = 2 * np.pi * ((n * k) % 128) / 128
    C, Sn = np.cos(a2), np.sin(a2)
    mf = np.block([[C, -Sn], [Sn, C]]); mi = np.block([[C, Sn], [-Sn, C]])
    k1 = np.arange(16)[:, None]; n2 = np.arange(128)[None, :]
    a3 = 2 * np.pi * (k1 * n2) / S
    tw = np.concatenate([np.repeat(np.cos(a3), 8, 0), np.repeat(np.sin(a3), 8, 0)], 0)
    return (ft.astype(nb), gt.astype(nb), np.concatenate([mf, mi], 0).astype(nb), tw.astype(np.float32))
FT, GT, MM, TW = _consts()

def dot(a, b, dn=NN):
    return lax.dot_general(a, b, dn, preferred_element_type=f32)

def _dft4(x0, x1, x2, x3, sg):
    t0 = (x0[0] + x2[0], x0[1] + x2[1]); t1 = (x0[0] - x2[0], x0[1] - x2[1])
    t2 = (x1[0] + x3[0], x1[1] + x3[1]); t3 = (x1[0] - x3[0], x1[1] - x3[1])
    X0 = (t0[0] + t2[0], t0[1] + t2[1]); X2 = (t0[0] - t2[0], t0[1] - t2[1])
    if sg < 0:
        X1 = (t1[0] + t3[1], t1[1] - t3[0]); X3 = (t1[0] - t3[1], t1[1] + t3[0])
    else:
        X1 = (t1[0] - t3[1], t1[1] + t3[0]); X3 = (t1[0] + t3[1], t1[1] - t3[0])
    return X0, X1, X2, X3

def _rot16(x, e, sg):
    e = e % 16
    a, b = x
    if e == 0: return x
    if e == 4: return (-b, a) if sg > 0 else (b, -a)
    c = float(np.cos(2 * np.pi * e / 16)); s = float(sg * np.sin(2 * np.pi * e / 16))
    if e % 2 == 0:
        if c * s > 0: return ((a - b) * c, (a + b) * c)
        return ((a + b) * c, (b - a) * c)
    return (a * c - b * s, a * s + b * c)

def fft16(xs, sg):
    u = [_dft4(xs[b], xs[4 + b], xs[8 + b], xs[12 + b], sg) for b in range(4)]
    out = [None] * 16
    for c in range(4):
        v = [_rot16(u[b][c], b * c, sg) for b in range(4)]
        r = _dft4(v[0], v[1], v[2], v[3], sg)
        for d in range(4):
            out[c + 4 * d] = r[d]
    return out

SLABS = [(r, 16) for r in range(0, 288, 16)] + [(288, 8)]

def interleave(main, side):
    n, m = len(main), len(side); k = 0
    for i, f in enumerate(main):
        f()
        while k < m and (k + 1) * n <= (i + 1) * m:
            side[k](); k += 1
    while k < m:
        side[k](); k += 1

def kern(xa_h, wr_h, wi_h, xb_h, w_h, wo_h, ft_h, gt_h, mm_h, tw_h, out_h,
         xa, wr, wi, xb, w, wo, ft, gt, mm, tw, yr, yi, wn, wpr, wpi, ytail, ob, kp, qt, vt, ot, sem):
    nsem = [0]
    def cp(a, b):
        c = pltpu.make_async_copy(a, b, sem.at[nsem[0]]); nsem[0] += 1
        return c
    XC = [(0, 256), (256, 256), (512, 512), (1024, 512), (1536, 512)]
    c_ft = cp(ft_h, ft)
    c_xa = [cp(xa_h.at[:, pl.ds(a, n_)], xa.at[:, pl.ds(a, n_)]) for a, n_ in XC]
    c_tw, c_w, c_xb, c_mm, c_wr, c_wi, c_gt, c_wo = [cp(a, b) for a, b in
        [(tw_h, tw), (w_h, w), (xb_h, xb), (mm_h, mm), (wr_h, wr), (wi_h, wi), (gt_h, gt), (wo_h, wo)]]
    c_ft.start(); c_xa[0].start(); c_xa[1].start()

    c_ft.wait()
    later = {0: [c_xa[2], c_w], 1: [c_xa[3]], 2: [c_xa[4], c_xb], 3: [c_tw, c_wr, c_wi], 4: [c_mm, c_gt, c_wo]}
    for c, (a, n_) in enumerate(XC):
        c_xa[c].wait()
        for x_ in later[c]: x_.start()
        y = dot(ft[...], xa[:, a:a+n_])
        yr[:, a:a+n_] = y[0:FP]
        yi[:, a:a+n_] = y[FP:2*FP]

    def twid(k1, nr):
        c_ = tw[k1*8:(k1+1)*8, :]; s_ = tw[128 + k1*8:128 + (k1+1)*8, :]
        if nr == 16:
            c_ = jnp.concatenate([c_, c_], 0); s_ = jnp.concatenate([s_, s_], 0)
        return c_, s_
    def a2(r0, nr):
        xs = [(yr[r0:r0+nr, t*128:(t+1)*128], yi[r0:r0+nr, t*128:(t+1)*128]) for t in range(16)]
        a = fft16(xs, -1)
        for k1 in range(16):
            re, im = a[k1]
            if k1 > 0:
                c_, s_ = twid(k1, nr)
                re, im = re * c_ + im * s_, im * c_ - re * s_
            yr[r0:r0+nr, k1*128:(k1+1)*128] = re
            yi[r0:r0+nr, k1*128:(k1+1)*128] = im
    def a3a(src, rb):
        if rb < 2:
            blk = src[rb*128:(rb+1)*128, :].astype(f32)
        else:
            blk = jnp.concatenate([src[256:DF, :].astype(f32), jnp.zeros((384 - DF, S), f32)], 0)
        wn[rb] = blk.T
    def a3b(dst, k1):
        for rb in range(3):
            t_ = wn[rb, pl.ds(k1, 128, stride=16), :].T
            if rb < 2:
                dst[rb*128:(rb+1)*128, k1*128:(k1+1)*128] = t_
            else:
                dst[256:FP, k1*128:(k1+1)*128] = t_[0:FP-256]
    def a4(k1):
        sl = slice(k1*128, (k1+1)*128)
        b = jnp.concatenate([yr[:, sl], yi[:, sl]], 1)
        x = dot(b, mm[0:256, :])
        xr, xi = x[:, 0:128], x[:, 128:256]
        a_, b_ = wpr[:, sl], wpi[:, sl]
        z = jnp.concatenate([xr * a_ - xi * b_, xr * b_ + xi * a_], 1)
        y = dot(z, mm[256:512, :])
        yr[:, sl] = y[:, 0:128]
        yi[:, sl] = y[:, 128:256]
    def a5(r0, nr):
        xs = []
        for k1 in range(16):
            re = yr[r0:r0+nr, k1*128:(k1+1)*128]; im = yi[r0:r0+nr, k1*128:(k1+1)*128]
            if k1 > 0:
                c_, s_ = twid(k1, nr)
                re, im = re * c_ - im * s_, im * c_ + re * s_
            xs.append((re, im))
        a = fft16(xs, +1)
        for t in range(16):
            yr[r0:r0+nr, t*128:(t+1)*128] = a[t][0]
            yi[r0:r0+nr, t*128:(t+1)*128] = a[t][1]
    def a6(c):
        sl = slice(c*512, (c+1)*512)
        z = jnp.concatenate([yr[:, sl], yi[:, sl]], 0).astype(bf)
        y = dot(gt[...], z).astype(bf)
        ob[sl, 0:512] = y[0:512].T
        ytail[:, sl] = y[512:576]

    zpad = jnp.zeros((D, 56), bf)
    def win(base, g):
        if g < 4: return w[:, base + 126*g : base + 126*g + 128]
        return jnp.concatenate([w[:, base + 504 : base + 576], zpad], 1)
    mx = {"q": jnp.zeros((8, 512), f32), "k": jnp.zeros((8, 512), f32), "v": jnp.zeros((8, 512), f32)}
    wts = {}
    def amax(key, v):
        acc = mx[key]
        for r in range(v.shape[0] // 8):
            acc = jnp.maximum(acc, jnp.abs(v[r*8:(r+1)*8]))
        mx[key] = acc
    def qi(g, c):
        if c == 0: wts["q"] = win(0, g).T
        sl = slice(c*512, (c+1)*512)
        q = (dot(wts["q"], xb[:, sl]) * CQ).astype(bf)
        qt[g*128:(g+1)*128, sl] = q
        amax("q", q.astype(f32))
    def ki(g, c):
        if c == 0: wts["k"] = win(D, g).T
        sl = slice(c*512, (c+1)*512)
        k = dot(wts["k"], xb[:, sl]).astype(bf)
        amax("k", k.astype(f32))
        kp[sl, g*128:(g+1)*128] = k.T
    def vi(g, c):
        if c == 0: wts["v"] = w[:, 2*D + 192*g : 2*D + 192*(g+1)].T
        sl = slice(c*512, (c+1)*512)
        v = dot(wts["v"], xb[:, sl])
        amax("v", v)
        vt[192*g:192*(g+1), sl] = v
    P = functools.partial
    q_items = [P(qi, g, c) for g in range(5) for c in range(4)]
    k_items = [P(ki, g, c) for g in range(5) for c in range(4)]
    v_items = [P(vi, g, c) for g in range(3) for c in range(4)]
    a2_items = [P(a2, r0, nr) for r0, nr in SLABS]
    a3_items = []
    for src, dst in ((wr, wpr), (wi, wpi)):
        a3_items += [P(a3a, src, rb) for rb in range(3)] + [P(a3b, dst, k1) for k1 in range(16)]
    a5_items = [P(a5, r0, nr) for r0, nr in SLABS]

    c_tw.wait(); c_w.wait(); c_xb.wait()
    interleave(q_items[:10], a2_items)
    c_wr.wait(); c_wi.wait(); c_mm.wait()
    interleave(q_items[10:] + k_items[:8], a3_items)
    for k1 in range(16): a4(k1)
    interleave(k_items[8:], a5_items)
    c_gt.wait()
    for c in range(4): a6(c)
    c_oa = cp(ob.at[:, pl.ds(0, 512)], out_h.at[:, pl.ds(0, 512)])
    c_oa.start()
    for f_ in v_items: f_()
    bound = jnp.max(mx["q"]) * jnp.max(mx["k"]) * DH
    vm = jnp.max(mx["v"])
    safe = (bound <= T_SAFE) & (vm <= 2.0**60) & ((vm >= 2.0**-60) | (vm == 0.0))
    ot[...] = jnp.zeros_like(ot)

    W = 512; ch = 128; n = S // ch; lag = 2
    def head_ids(h):
        g = h // 7
        j = h - 7 * g
        g128 = pl.multiple_of(g * 128, 128)
        w0 = pl.multiple_of((18 * h) // 8 * 8, 8)
        wr_ = lax.broadcasted_iota(jnp.int32, (64, W), 0)
        qmask = (wr_ >= 9 * j) & (wr_ < 9 * j + 9)
        rr = lax.broadcasted_iota(jnp.int32, (24, W), 0) + w0
        omask = (rr >= 18 * h) & (rr < 18 * h + 18)
        return g128, w0, qmask, omask
    def load_q(g128, qmask, q):
        qraw = pltpu.bitcast(qt[pl.ds(g128, 128), q*W:(q+1)*W], u32)
        return pltpu.bitcast(jnp.where(qmask, qraw, jnp.uint32(0)), bf)
    def core(h, mrow):
        g128, w0, qmask, omask = head_ids(h)
        steps = [(q, cc) for q in range(4) for cc in range(n)]
        ps = {}; accs = {}; ls = {}; qm = {}
        for t in range(len(steps) + lag):
            if t < len(steps):
                q, cc = steps[t]
                if cc == 0:
                    qm[q] = load_q(g128, qmask, q)
                s = dot(kp[cc*ch:(cc+1)*ch, pl.ds(g128, 128)], qm[q])
            if t >= lag:
                q2, c2 = steps[t - lag]
                r = dot(vt[pl.ds(w0, 24), c2*ch:(c2+1)*ch], ps.pop(t - lag))
                accs[q2] = r if c2 == 0 else accs[q2] + r
                if c2 == n - 1:
                    a = accs.pop(q2)
                    l = jnp.sum(ls.pop(q2), axis=0, keepdims=True)
                    o = a * (1.0 / l)
                    old = ot[pl.ds(w0, 24), q2*W:(q2+1)*W]
                    ot[pl.ds(w0, 24), q2*W:(q2+1)*W] = jnp.where(omask, o, old)
            if t < len(steps):
                if mrow is not None:
                    s = s - mrow[q]
                p = jnp.exp2(s)
                l = p[0:8]
                for r8 in range(1, ch // 8):
                    l = l + p[r8*8:(r8+1)*8]
                ls[q] = l if cc == 0 else ls[q] + l
                ps[t] = p.astype(bf)
    def head_fast(h, carry):
        core(h, None)
        return carry
    def head_slow(h, carry):
        g128, w0, qmask, omask = head_ids(h)
        mrow = []
        for q in range(4):
            qm = load_q(g128, qmask, q)
            def mx(cc, m):
                c0 = pl.multiple_of(cc * 256, 256)
                s = dot(kp[pl.ds(c0, 256), pl.ds(g128, 128)], qm)
                for r8 in range(32):
                    m = jnp.maximum(m, s[r8*8:(r8+1)*8])
                return m
            m = lax.fori_loop(0, S // 256, mx, jnp.full((8, W), -jnp.inf, f32))
            mrow.append(jnp.max(m, axis=0, keepdims=True))
        core(h, mrow)
        return carry
    @pl.when(safe)
    def _():
        lax.fori_loop(0, H, head_fast, 0)
    @pl.when(jnp.logical_not(safe))
    def _():
        lax.fori_loop(0, H, head_slow, 0)

    c_wo.wait()
    wot = wo[...].T
    outs = [c_oa]
    OC = [(0, 512), (512, 512), (1024, 512), (1536, 256), (1792, 256)]
    for a, n_ in OC:
        sl = slice(a, a + n_)
        b = dot(wot, ot[:, sl].astype(bf)).astype(bf)
        ob[sl, 512:1152] = jnp.concatenate([ytail[:, sl], b], 0).T
        c = cp(ob.at[pl.ds(a, n_), pl.ds(512, 640)], out_h.at[pl.ds(a, n_), pl.ds(512, 640)])
        c.start(); outs.append(c)
    for c in outs: c.wait()

@jax.jit
def pallas_concat_heads__spectral_gfnet__mha_block__prompt_kernel(A_x, A_w_r, A_w_i, B_x, B_wqkv, B_wo):
    V = pltpu.VMEM
    scratch = [V((D, S), bf), V((DF, S), bf), V((DF, S), bf), V((D, S), bf), V((D, 3*D), bf), V((D, D), bf),
               V(FT.shape, bf), V(GT.shape, bf), V(MM.shape, bf), V(TW.shape, f32),
               V((FP, S), f32), V((FP, S), f32), V((3, S, 128), f32), V((FP, S), f32), V((FP, S), f32),
               V((64, S), bf), V((S, 2*D), bf), V((S, 640), bf), V((640, S), bf), V((D, S), f32), V((D, S), f32),
               pltpu.SemaphoreType.DMA((24,))]
    anyspec = pl.BlockSpec(memory_space=pl.ANY)
    out = pl.pallas_call(kern, out_shape=jax.ShapeDtypeStruct((S, 2*D), bf),
        in_specs=[anyspec]*10, out_specs=anyspec, scratch_shapes=scratch,
        compiler_params=pltpu.CompilerParams(vmem_limit_bytes=110*1024*1024), name="full2")(
        A_x[0].T, A_w_r.T, A_w_i.T, B_x[0].T, B_wqkv, B_wo, FT, GT, MM, TW)
    return out[None]
```

```python
import functools
import numpy as np, jax, jax.numpy as jnp, ml_dtypes
from jax import lax
from jax.experimental import pallas as pl
from jax.experimental.pallas import tpu as pltpu

f32 = jnp.float32; bf = jnp.bfloat16; u32 = jnp.uint32
S, D, H, DH = 2048, 576, 32, 18
DF = D // 2 + 1
FE, FO = 152, 144
FP = 296
NN = (((1,), (0,)), ((), ()))
CQ = float(DH ** -0.5 * np.log2(np.e))
T_SAFE = 40.0

def _consts():
    nb = ml_dtypes.bfloat16
    hd = D // 2
    d = np.arange(hd)[None, :].astype(np.float64)
    fe = np.arange(0, DF, 2)[:, None].astype(np.float64); fo = np.arange(1, DF, 2)[:, None].astype(np.float64)
    ae = 2 * np.pi * ((fe * d) % D) / D; ao = 2 * np.pi * ((fo * d) % D) / D
    ft = np.zeros((2 * FP, hd))
    ft[0:145] = np.cos(ae); ft[FE:FE + 145] = -np.sin(ae)
    ft[2 * FE:2 * FE + FO] = np.cos(ao); ft[2 * FE + FO:] = -np.sin(ao)
    cf = np.full((2 * FP, 1), 2.0); cf[0] = 1.0; cf[144] = 1.0
    g_ = (cf * ft).T / (D * S)
    gt = np.zeros((hd, 768)); gt[:, 0:2 * FE] = g_[:, 0:2 * FE]; gt[:, 384:384 + 2 * FO] = g_[:, 2 * FE:]
    n = np.arange(128)[:, None].astype(np.float64); k = np.arange(128)[None, :].astype(np.float64)
    a2 = 2 * np.pi * ((n * k) % 128) / 128
    C, Sn = np.cos(a2), np.sin(a2)
    mf = np.concatenate([C, -Sn - C, C - Sn], 0); mi = np.concatenate([C, Sn - C, C + Sn], 0)
    k1 = np.arange(16)[:, None]; n2 = np.arange(128)[None, :]
    a3 = 2 * np.pi * (k1 * n2) / S
    tw = np.concatenate([np.repeat(np.cos(a3), 8, 0), np.repeat(np.sin(a3), 8, 0)], 0)
    return (ft.astype(nb), gt.astype(nb), np.concatenate([mf, mi], 0).astype(nb), tw.astype(np.float32))
FT, GT, MM, TW = _consts()

def dot(a, b, dn=NN):
    return lax.dot_general(a, b, dn, preferred_element_type=f32)

def _dft4(x0, x1, x2, x3, sg):
    t0 = (x0[0] + x2[0], x0[1] + x2[1]); t1 = (x0[0] - x2[0], x0[1] - x2[1])
    t2 = (x1[0] + x3[0], x1[1] + x3[1]); t3 = (x1[0] - x3[0], x1[1] - x3[1])
    X0 = (t0[0] + t2[0], t0[1] + t2[1]); X2 = (t0[0] - t2[0], t0[1] - t2[1])
    if sg < 0:
        X1 = (t1[0] + t3[1], t1[1] - t3[0]); X3 = (t1[0] - t3[1], t1[1] + t3[0])
    else:
        X1 = (t1[0] - t3[1], t1[1] + t3[0]); X3 = (t1[0] + t3[1], t1[1] - t3[0])
    return X0, X1, X2, X3

def _rot16(x, e, sg):
    e = e % 16
    a, b = x
    if e == 0: return x
    if e == 4: return (-b, a) if sg > 0 else (b, -a)
    c = float(np.cos(2 * np.pi * e / 16)); s = float(sg * np.sin(2 * np.pi * e / 16))
    if e % 2 == 0:
        if c * s > 0: return ((a - b) * c, (a + b) * c)
        return ((a + b) * c, (b - a) * c)
    return (a * c - b * s, a * s + b * c)

def fft16(xs, sg):
    u = [_dft4(xs[b], xs[4 + b], xs[8 + b], xs[12 + b], sg) for b in range(4)]
    out = [None] * 16
    for c in range(4):
        v = [_rot16(u[b][c], b * c, sg) for b in range(4)]
        r = _dft4(v[0], v[1], v[2], v[3], sg)
        for d in range(4):
            out[c + 4 * d] = r[d]
    return out

SLABS = [(r, 16) for r in range(0, 288, 16)] + [(288, 8)]

def interleave(main, side):
    n, m = len(main), len(side); k = 0
    for i, f in enumerate(main):
        f()
        while k < m and (k + 1) * n <= (i + 1) * m:
            side[k](); k += 1
    while k < m:
        side[k](); k += 1

def kern(xa_h, wr_h, wi_h, xb_h, w_h, wo_h, ft_h, gt_h, mm_h, tw_h, out_h,
         xa, wr, wi, xb, w, wo, ft, gt, mm, tw, yr, yi, wn, wpr, wpi, ytail, ob, kt, kp, qt, vt, ot, sem):
    nsem = [0]
    def cp(a, b):
        c = pltpu.make_async_copy(a, b, sem.at[nsem[0]]); nsem[0] += 1
        return c
    XC = [(0, 256), (256, 256), (512, 512), (1024, 512), (1536, 512)]
    c_ft = cp(ft_h, ft)
    c_xa = [cp(xa_h.at[:, pl.ds(a, n_)], xa.at[:, pl.ds(a, n_)]) for a, n_ in XC]
    c_tw, c_w, c_xb, c_mm, c_wr, c_wi, c_gt, c_wo = [cp(a, b) for a, b in
        [(tw_h, tw), (w_h, w), (xb_h, xb), (mm_h, mm), (wr_h, wr), (wi_h, wi), (gt_h, gt), (wo_h, wo)]]
    c_ft.start(); c_xa[0].start(); c_xa[1].start()

    c_ft.wait()
    later = {0: [c_xa[2], c_xa[3]], 1: [c_xa[4], c_w], 2: [c_xb], 3: [c_tw, c_wr, c_wi], 4: [c_mm, c_gt, c_wo]}
    for c, (a, n_) in enumerate(XC):
        c_xa[c].wait()
        for x_ in later[c]: x_.start()
        x0 = xa[0:D//2, a:a+n_].astype(f32); x1 = xa[D//2:D, a:a+n_].astype(f32)
        y = dot(ft[0:2*FE, :], (x0 + x1).astype(bf))
        yr[0:FE, a:a+n_] = y[0:FE]
        yi[0:FE, a:a+n_] = y[FE:2*FE]
        y = dot(ft[2*FE:2*FP, :], (x0 - x1).astype(bf))
        yr[FE:FP, a:a+n_] = y[0:FO]
        yi[FE:FP, a:a+n_] = y[FO:2*FO]

    def twid(k1, nr):
        c_ = tw[k1*8:(k1+1)*8, :]; s_ = tw[128 + k1*8:128 + (k1+1)*8, :]
        if nr == 16:
            c_ = jnp.concatenate([c_, c_], 0); s_ = jnp.concatenate([s_, s_], 0)
        return c_, s_
    def a2(r0, nr):
        xs = [(yr[r0:r0+nr, t*128:(t+1)*128], yi[r0:r0+nr, t*128:(t+1)*128]) for t in range(16)]
        a = fft16(xs, -1)
        for k1 in range(16):
            re, im = a[k1]
            if k1 > 0:
                c_, s_ = twid(k1, nr)
                re, im = re * c_ + im * s_, im * c_ - re * s_
            yr[r0:r0+nr, k1*128:(k1+1)*128] = re
            yi[r0:r0+nr, k1*128:(k1+1)*128] = im
    def a3a(src, rb):
        if rb < 2:
            blk = src[rb*128:(rb+1)*128, :].astype(f32)
        else:
            blk = jnp.concatenate([src[256:DF, :].astype(f32), jnp.zeros((384 - DF, S), f32)], 0)
        wn[rb] = blk.T
    def a3b(dst, k1):
        for rb in range(3):
            t_ = wn[rb, pl.ds(k1, 128, stride=16), :].T
            if rb < 2:
                dst[k1, rb*128:(rb+1)*128, :] = t_
            else:
                dst[k1, 256:304, :] = t_[0:48]
    def a4(k1):
        sl = slice(k1*128, (k1+1)*128)
        def cmm(a, b, o):
            t1 = dot(a + b, mm[o:o+128, :]); t2 = dot(a, mm[o+128:o+256, :]); t3 = dot(b, mm[o+256:o+384, :])
            return t1 - t3, t1 + t2
        xr, xi = cmm(yr[:, sl], yi[:, sl], 0)
        a_ = jnp.concatenate([wpr[k1, pl.ds(0, FE, stride=2), :], wpr[k1, pl.ds(1, FO, stride=2), :]], 0)
        b_ = jnp.concatenate([wpi[k1, pl.ds(0, FE, stride=2), :], wpi[k1, pl.ds(1, FO, stride=2), :]], 0)
        zr, zi = cmm(xr * a_ - xi * b_, xr * b_ + xi * a_, 384)
        yr[:, sl] = zr
        yi[:, sl] = zi
    def a5(r0, nr):
        xs = []
        for k1 in range(16):
            re = yr[r0:r0+nr, k1*128:(k1+1)*128]; im = yi[r0:r0+nr, k1*128:(k1+1)*128]
            if k1 > 0:
                c_, s_ = twid(k1, nr)
                re, im = re * c_ - im * s_, im * c_ + re * s_
            xs.append((re, im))
        a = fft16(xs, +1)
        for t in range(16):
            yr[r0:r0+nr, t*128:(t+1)*128] = a[t][0]
            yi[r0:r0+nr, t*128:(t+1)*128] = a[t][1]
    def a6(c):
        sl = slice(c*512, (c+1)*512)
        ze = jnp.concatenate([yr[0:FE, sl], yi[0:FE, sl]], 0).astype(bf)
        zo = jnp.concatenate([yr[FE:FP, sl], yi[FE:FP, sl]], 0).astype(bf)
        ya = dot(gt[:, 0:2*FE], ze); yb = dot(gt[:, 384:384+2*FO], zo)
        y = jnp.concatenate([ya + yb, ya - yb], 0).astype(bf)
        ob[sl, 0:512] = y[0:512].T
        ytail[:, sl] = y[512:576]

    mx = {"q": jnp.zeros((8, 512), f32), "k": jnp.zeros((8, 512), f32), "v": jnp.zeros((8, 512), f32)}
    wts = {}
    def amax(key, v):
        acc = mx[key]
        for r in range(v.shape[0] // 8):
            acc = jnp.maximum(acc, jnp.abs(v[r*8:(r+1)*8]))
        mx[key] = acc
    def qi(g, c):
        if c == 0: wts["q"] = w[:, 192*g : 192*(g+1)].T
        sl = slice(c*512, (c+1)*512)
        q = (dot(wts["q"], xb[:, sl]) * CQ).astype(bf)
        qt[192*g:192*(g+1), sl] = q
        amax("q", q.astype(f32))
    def ki(g, c):
        if c == 0: wts["k"] = w[:, D + 192*g : D + 192*(g+1)].T
        sl = slice(c*512, (c+1)*512)
        k = dot(wts["k"], xb[:, sl]).astype(bf)
        amax("k", k.astype(f32))
        kt[192*g:192*(g+1), sl] = k
    def kx(g, c):
        a = min(108 * g // 16 * 16, D - 128)
        kp[c*512:(c+1)*512, g*128:(g+1)*128] = kt[a:a+128, c*512:(c+1)*512].T
    def vi(g, c):
        if c == 0: wts["v"] = w[:, 2*D + 192*g : 2*D + 192*(g+1)].T
        sl = slice(c*512, (c+1)*512)
        v = dot(wts["v"], xb[:, sl])
        amax("v", v)
        vt[192*g:192*(g+1), sl] = v
    P = functools.partial
    q_items = [P(qi, g, c) for g in range(3) for c in range(4)]
    k_items = [P(ki, g, c) for g in range(3) for c in range(4)]
    kx_items = [P(kx, g, c) for g in range(6) for c in range(4)]
    v_items = [P(vi, g, c) for g in range(3) for c in range(4)]
    a2_items = [P(a2, r0, nr) for r0, nr in SLABS]
    a3_items = []
    for src, dst in ((wr, wpr), (wi, wpi)):
        a3_items += [P(a3a, src, rb) for rb in range(3)] + [P(a3b, dst, k1) for k1 in range(16)]
    a5_items = [P(a5, r0, nr) for r0, nr in SLABS]

    ot[...] = jnp.zeros_like(ot)
    c_tw.wait(); c_w.wait(); c_xb.wait()
    interleave(q_items[:6], a2_items)
    c_wr.wait(); c_wi.wait(); c_mm.wait()
    interleave(q_items[6:] + k_items[:6], a3_items)
    for k1 in range(16): a4(k1)
    interleave(k_items[6:], a5_items[:8])
    interleave(v_items, a5_items[8:] + kx_items)
    bound = jnp.max(mx["q"]) * jnp.max(mx["k"]) * DH
    vm = jnp.max(mx["v"])
    safe = (bound <= T_SAFE) & (vm <= 2.0**60) & ((vm >= 2.0**-60) | (vm == 0.0))

    W = 512; ch = 128; n = S // ch; lag = 2
    def head_ids(h):
        g = h // 6
        g128 = pl.multiple_of(g * 128, 128)
        a0 = pl.multiple_of(jnp.minimum((108 * g) // 16 * 16, D - 128), 16)
        j = 9 * h - a0 // 2
        w0 = pl.multiple_of((18 * h) // 8 * 8, 8)
        wr_ = lax.broadcasted_iota(jnp.int32, (64, W), 0)
        qmask = (wr_ >= j) & (wr_ < j + 9)
        rr = lax.broadcasted_iota(jnp.int32, (24, W), 0) + w0
        omask = (rr >= 18 * h) & (rr < 18 * h + 18)
        return (g128, a0), w0, qmask, omask
    def load_q(g128, qmask, q):
        qraw = pltpu.bitcast(qt[pl.ds(g128[1], 128), q*W:(q+1)*W], u32)
        return pltpu.bitcast(jnp.where(qmask, qraw, jnp.uint32(0)), bf)
    def core(h, mrow):
        g128, w0, qmask, omask = head_ids(h)
        steps = [(q, cc) for q in range(4) for cc in range(n)]
        ps = {}; accs = {}; ls = {}; qm = {}
        for t in range(len(steps) + lag):
            if t < len(steps):
                q, cc = steps[t]
                if cc == 0:
                    qm[q] = load_q(g128, qmask, q)
                s = dot(kp[cc*ch:(cc+1)*ch, pl.ds(g128[0], 128)], qm[q])
            if t >= lag:
                q2, c2 = steps[t - lag]
                r = dot(vt[pl.ds(w0, 24), c2*ch:(c2+1)*ch], ps.pop(t - lag))
                accs[q2] = r if c2 == 0 else accs[q2] + r
                if c2 == n - 1:
                    a = accs.pop(q2)
                    l = jnp.sum(ls.pop(q2), axis=0, keepdims=True)
                    o = a * (1.0 / l)
                    old = ot[pl.ds(w0, 24), q2*W:(q2+1)*W]
                    ot[pl.ds(w0, 24), q2*W:(q2+1)*W] = jnp.where(omask, o, old)
            if t < len(steps):
                if mrow is not None:
                    s = s - mrow[q]
                p = jnp.exp2(s)
                l = p[0:8]
                for r8 in range(1, ch // 8):
                    l = l + p[r8*8:(r8+1)*8]
                ls[q] = l if cc == 0 else ls[q] + l
                ps[t] = p.astype(bf)
    UN = 2
    def head_fast(i, carry):
        for u in range(UN):
            core(i * UN + u, None)
        return carry
    def head_slow(h, carry):
        g128, w0, qmask, omask = head_ids(h)
        mrow = []
        for q in range(4):
            qm = load_q(g128, qmask, q)
            def mx(cc, m):
                c0 = pl.multiple_of(cc * 256, 256)
                s = dot(kp[pl.ds(c0, 256), pl.ds(g128[0], 128)], qm)
                for r8 in range(32):
                    m = jnp.maximum(m, s[r8*8:(r8+1)*8])
                return m
            m = lax.fori_loop(0, S // 256, mx, jnp.full((8, W), -jnp.inf, f32))
            mrow.append(jnp.max(m, axis=0, keepdims=True))
        core(h, mrow)
        return carry
    @pl.when(safe)
    def _():
        lax.fori_loop(0, H // UN, head_fast, 0)
    @pl.when(jnp.logical_not(safe))
    def _():
        lax.fori_loop(0, H, head_slow, 0)

    c_gt.wait()
    outs = []
    for c in range(4):
        a6(c)
        cc_ = cp(ob.at[pl.ds(c*512, 512), pl.ds(0, 512)], out_h.at[pl.ds(c*512, 512), pl.ds(0, 512)])
        cc_.start(); outs.append(cc_)
    c_wo.wait()
    wot = wo[...].T
    OC = [(0, 512), (512, 512), (1024, 512), (1536, 256), (1792, 256)]
    for a, n_ in OC:
        sl = slice(a, a + n_)
        b = dot(wot, ot[:, sl].astype(bf)).astype(bf)
        ob[sl, 512:1152] = jnp.concatenate([ytail[:, sl], b], 0).T
        c = cp(ob.at[pl.ds(a, n_), pl.ds(512, 640)], out_h.at[pl.ds(a, n_), pl.ds(512, 640)])
        c.start(); outs.append(c)
    for c in outs: c.wait()

@jax.jit
def pallas_concat_heads__spectral_gfnet__mha_block__prompt_kernel(A_x, A_w_r, A_w_i, B_x, B_wqkv, B_wo):
    V = pltpu.VMEM
    scratch = [V((D, S), bf), V((DF, S), bf), V((DF, S), bf), V((D, S), bf), V((D, 3*D), bf), V((D, D), bf),
               V(FT.shape, bf), V(GT.shape, bf), V(MM.shape, bf), V(TW.shape, f32),
               V((FP, S), f32), V((FP, S), f32), V((3, S, 128), f32), V((16, 304, 128), f32), V((16, 304, 128), f32),
               V((64, S), bf), V((S, 2*D), bf), V((D, S), bf), V((S, 768), bf), V((D, S), bf), V((D, S), f32), V((D, S), f32),
               pltpu.SemaphoreType.DMA((24,))]
    anyspec = pl.BlockSpec(memory_space=pl.ANY)
    out = pl.pallas_call(kern, out_shape=jax.ShapeDtypeStruct((S, 2*D), bf),
        in_specs=[anyspec]*10, out_specs=anyspec, scratch_shapes=scratch,
        compiler_params=pltpu.CompilerParams(vmem_limit_bytes=110*1024*1024), name="gfnet_mha")(
        A_x[0].T, A_w_r.T, A_w_i.T, B_x[0].T, B_wqkv, B_wo, FT, GT, MM, TW)
    return out[None]
```
